```python
import os as _os
_os.environ.setdefault("JAX_PLATFORMS", "cpu")
import jax
import jax.numpy as jnp

def _softmax(x, axis=-1):
    return jax.nn.softmax(x, axis=axis)
def _gelu(x):
    return jax.nn.gelu(x, approximate=True)
def _silu(x):
    return jax.nn.silu(x)
def _sigmoid(x):
    return jax.nn.sigmoid(x)
def _layernorm(x, axis=-1, eps=1e-5):
    m = jnp.mean(x, axis=axis, keepdims=True)
    v = jnp.var(x, axis=axis, keepdims=True)
    return (x - m) / jnp.sqrt(v + eps)
def _scatter_add(tgt, idx, src, axis=0):
    return tgt.at[idx].add(src)
def _segment_sum(src, seg, n):
    return jax.ops.segment_sum(src, seg, n)
class _Rng:
    def __init__(self, key):
        self._k = key
    def _next(self):
        self._k, sub = jax.random.split(self._k)
        return sub
    def normal(self, shape):
        return jax.random.normal(self._next(), shape, dtype=jnp.bfloat16)
    def randint(self, lo, hi, shape):
        return jax.random.randint(self._next(), shape, lo, hi, dtype=jnp.int32)
    def uniform(self, shape, lo=0.0, hi=1.0):
        return jax.random.uniform(self._next(), shape, jnp.bfloat16, lo, hi)
    def permutation(self, n):
        return jax.random.permutation(self._next(), n)


kernel_name = 'interleave_layers__sliding_local_dilated__sliding_local_dilated__prompt'

def setup_inputs():
    _rng = _Rng(jax.random.key(int.from_bytes(__import__("os").urandom(4), "little")))
    _w = (lambda a: (lambda t: t.astype(jnp.bfloat16) if jnp.issubdtype(t.dtype, jnp.floating) else t)(jnp.asarray(a)))
    def _A_setup():
        B, S, D = 1, 2048, 1024
        return {
            "x": _w((lambda *s: _rng.normal(s) * 0.05)(B, S, D)),
            "wqkv": _w((lambda *s: _rng.normal(s) * 0.05)(D, 3 * D)),
            "wo": _w((lambda *s: _rng.normal(s) * 0.05)(D, D)),
        }
    _A_in = _A_setup()

    def _B_setup():
        B, S, D = 1, 2048, 1024
        return {
            "x": _w((lambda *s: _rng.normal(s) * 0.05)(B, S, D)),
            "wqkv": _w((lambda *s: _rng.normal(s) * 0.05)(D, 3 * D)),
            "wo": _w((lambda *s: _rng.normal(s) * 0.05)(D, D)),
        }
    _B_in = _B_setup()

    return {
        "A_x": _A_in["x"],
        "A_wqkv": _A_in["wqkv"],
        "A_wo": _A_in["wo"],
        "B_x": _B_in["x"],
        "B_wqkv": _B_in["wqkv"],
        "B_wo": _B_in["wo"],
    }

def reference(A_x, A_wqkv, A_wo, B_x, B_wqkv, B_wo):
    def _A_ref(x, wqkv, wo):
        B, S, D = x.shape
        H = 32; Dh = D // H
        W, dil = 8, 2
        qkv = (lambda x, *d: x.transpose(*d))((x @ wqkv).reshape(B, S, 3, H, Dh), 2, 0, 3, 1, 4)
        q, k, v = qkv[0], qkv[1], qkv[2]
        scale = Dh ** -0.5
        pos = jnp.arange(S)
        off = jnp.arange(W) * dil
        idx = pos[:, None] - off[None, :]
        mask = idx >= 0
        idx_c = jnp.where(mask, idx, 0).reshape(-1)
        kg = k[:, :, idx_c, :].reshape(B, H, S, W, Dh)
        vg = v[:, :, idx_c, :].reshape(B, H, S, W, Dh)
        logits = jnp.einsum("bhsd,bhswd->bhsw", q, kg) * scale
        logits = jnp.where(mask[None, None, :, :], logits, -1e9)
        attn = _softmax(logits, axis=-1)
        o = jnp.einsum("bhsw,bhswd->bhsd", attn, vg)
        return (lambda x, *d: x.transpose(*d))(o, 0, 2, 1, 3).reshape(B, S, D) @ wo

    def _B_ref(x, wqkv, wo):
        B, S, D = x.shape
        H = 32; Dh = D // H
        W, dil = 8, 2
        qkv = (lambda x, *d: x.transpose(*d))((x @ wqkv).reshape(B, S, 3, H, Dh), 2, 0, 3, 1, 4)
        q, k, v = qkv[0], qkv[1], qkv[2]
        scale = Dh ** -0.5
        pos = jnp.arange(S)
        off = jnp.arange(W) * dil
        idx = pos[:, None] - off[None, :]
        mask = idx >= 0
        idx_c = jnp.where(mask, idx, 0).reshape(-1)
        kg = k[:, :, idx_c, :].reshape(B, H, S, W, Dh)
        vg = v[:, :, idx_c, :].reshape(B, H, S, W, Dh)
        logits = jnp.einsum("bhsd,bhswd->bhsw", q, kg) * scale
        logits = jnp.where(mask[None, None, :, :], logits, -1e9)
        attn = _softmax(logits, axis=-1)
        o = jnp.einsum("bhsw,bhswd->bhsd", attn, vg)
        return (lambda x, *d: x.transpose(*d))(o, 0, 2, 1, 3).reshape(B, S, D) @ wo

    x = A_x
    x = x + _A_ref(_layernorm(x, axis=-1), A_wqkv, A_wo)
    x = x + _B_ref(_layernorm(x, axis=-1), B_wqkv, B_wo)
    x = x + _A_ref(_layernorm(x, axis=-1), A_wqkv, A_wo)
    x = x + _B_ref(_layernorm(x, axis=-1), B_wqkv, B_wo)
    return x
```

```python
import os
EXP = os.environ.get('EXP','UV')
import functools
import jax
import numpy as np
import jax.numpy as jnp
import jax.experimental.pallas as pl
import jax.experimental.pallas.tpu as pltpu

S, D = 2048, 1024
H, DH = 32, 32
WIN = 8
NB = D // 128
TM = 256
NT = S // TM
NL = 4
NA = TM // 16
KP = (NA + WIN) * 8
NC = int(os.environ.get('NC', 256))
HI16, LO16 = np.uint32(0xFFFF0000), np.uint32(0xFFFF)
NQ = int(os.environ.get('NQ', 4))
QR = D // NQ
PREP_ROWS = int(os.environ.get('PREP', 128))
MX = [int(v) for v in os.environ.get('MX', '1357')]
MQ = [int(v) for v in os.environ.get('MQ', '1357')]
LN_EPS = 1e-5
SCALE = DH ** -0.5
LOG2E = 1.4426950408889634
F32, BF16, U32, I32 = jnp.float32, jnp.bfloat16, jnp.uint32, jnp.int32


def _token(words):
    return functools.reduce(jnp.bitwise_or, [
        w if w.shape == (8, 128) else w[a:a + 8, b:b + 128]
        for w in words for a in range(0, w.shape[0], 8) for b in range(0, w.shape[1], 128)])


def _aligned(v, m):
    return v if isinstance(v, int) else pl.multiple_of(v, m)


def _xor_shuffle(t, masks):
    t = list(t)
    for b, m in masks.items():
        for ia in range(len(t)):
            if not ia & b:
                lo, hi = t[ia], t[ia | b]
                t[ia], t[ia | b] = jnp.where(m, hi, lo), jnp.where(m, lo, hi)
    return t


def _lane_source(lane, j):
    dt, hh, hl = lane >> 5, (lane >> 2) & 7, lane & 3
    return hl * 32 + dt * 8 + (hh ^ j)


def _lane_matrix(j):
    src, lane = [jax.lax.broadcasted_iota(I32, (128, 128), axis) for axis in range(2)]
    return jnp.where(src == _lane_source(lane, j), 1.0, 0.0).astype(BF16)


def _permute_cols(blks, mats):
    lane = jax.lax.broadcasted_iota(I32, blks[0].shape, 1)
    t = _xor_shuffle(blks, {b: (lane & b) != 0 for b in (1, 2, 4)})
    return [
        pltpu.bitcast(jnp.dot(pltpu.bitcast(t[j], BF16), mats[j], preferred_element_type=F32).astype(BF16), I32)
        if j in mats else jnp.take_along_axis(t[j], _lane_source(lane, j), axis=1) for j in range(NB)]


def _transpose8(slabs):
    sub = jax.lax.broadcasted_iota(I32, slabs[0].shape, 0)
    t = list(slabs)
    for b in (1, 2, 4):
        m = (sub & b) != 0
        for ia in range(8):
            if not ia & b:
                lo, hi = t[ia], t[ia | b]
                t[ia] = jnp.where(m, pltpu.roll(hi, b, 0), lo)
                t[ia | b] = jnp.where(m, hi, pltpu.roll(lo, 8 - b, 0))
    return t


def _prep_wqkv(raw_ref, dst_ref, r0, rows, sec, mats=()):
    cols = pl.ds(_aligned(sec * D, D), D)
    raw = raw_ref.at[pl.ds(_aligned(2 * r0, 2 * rows), 2 * rows), cols]
    dst = dst_ref.at[pl.ds(_aligned(r0, rows), rows), cols]
    blks = _permute_cols([pltpu.bitcast(raw[:, j * 128:(j + 1) * 128], I32) for j in range(NB)], mats)
    blks = [pltpu.bitcast(blk, U32) for blk in blks]
    for j, blk in enumerate(blks):
        dst[:, j * 128:(j + 1) * 128] = blk
    return _token(blks)


def _prep_wo(raw_ref, dst_ref, part):
    cols = pl.ds(_aligned((part >> 2) * 128, 128), 128)
    h4, d4 = (part >> 1) & 1, part & 1
    raw = raw_ref.at[pl.ds(_aligned(h4 * (D // 2) + d4 * 16, 16), D // 2 - 16), cols]
    dst = [dst_ref.at[pl.ds(_aligned((h4 ^ d2) * 256 + d4 * 32 + h4 * 8, 8), 216), cols] for d2 in range(2)]
    sub = jax.lax.broadcasted_iota(I32, (8, 128), 0)
    ev, od = [_transpose8([pltpu.bitcast(raw[pl.ds((hm * 2 + h0) * DH, 16), :], U32) for hm in range(8)])
              for h0 in range(2)]
    words = []
    for dm in range(8):
        words += [(ev[dm] & LO16) | (od[dm] << 16), (ev[dm] >> 16) | (od[dm] & HI16)]
    words = _xor_shuffle(words, {1: (sub & 2) != 0, 2: (sub & 4) != 0})
    for n, word in enumerate(words):
        dst[(n >> 2) & 1][pl.ds((n & 3) * 64 + (n >> 3) * 16, 8), :] = word
    return _token(words)


def _load_x(src, dst):
    done = []
    for ah in range(NA // 8):
        t = _transpose8([pltpu.bitcast(src[pl.ds((s * (NA // 8) + ah) * 16, 16), :], U32) for s in range(8)])
        for al in range(8):
            a = ah * 8 + al
            dst[pl.ds(a * 8, 8), :] = pltpu.bitcast(t[al] << 16, F32)
            dst[pl.ds((NA + a) * 8, 8), :] = pltpu.bitcast(t[al] & HI16, F32)
        done += t
    return _token(done)


def _store_out(even, odd, dst, ah):
    words = pltpu.pack_elementwise([even, odd], packed_dtype=BF16)
    t = _transpose8([words[al * 8:(al + 1) * 8] for al in range(8)])
    for s in range(8):
        dst[pl.ds((s * (NA // 8) + ah) * 16, 16), :] = pltpu.bitcast(t[s], BF16)
    return _token(t)


def _ln_rows(x):
    m = jnp.mean(x, axis=-1, keepdims=True)
    c = x - m
    v = jnp.mean(c * c, axis=-1, keepdims=True)
    return c * jax.lax.rsqrt(v + LN_EPS)


def _attn_rows(q_ref, k_ref, v_ref, o_ref, par, a0, first):
    qr = (par * NA + a0) * 8
    kr = par * KP + (WIN + a0) * 8
    ls = [None] * WIN
    for j in range(NB):
        cols = pl.ds(j * 128, 128)
        q = q_ref[pl.ds(qr, 16), cols]
        for w in range(WIN):
            p = q * k_ref[pl.ds(kr - 8 * w, 16), cols]
            ls[w] = p if j == 0 else ls[w] + p
    row = jax.lax.broadcasted_iota(I32, (16, 128), 0)
    for w in range(WIN):
        l = ls[w]
        l = l + pltpu.roll(l, 64, 1)
        l = l + pltpu.roll(l, 32, 1)
        if w > a0 and first is not False:
            hit = (row == 0) if w == a0 + 1 else ((row & 7) == 0)
            l = jnp.where(jnp.logical_and(hit, first), -1e9 / SCALE, l)
        ls[w] = l
    m = ls[0]
    for w in range(1, WIN):
        m = jnp.maximum(m, ls[w])
    es = [jnp.exp2((l - m) * (SCALE * LOG2E)) for l in ls]
    den = es[0]
    for w in range(1, WIN):
        den = den + es[w]
    inv = 1.0 / den
    done = []
    if 'P' in EXP:
        es = [e * inv for e in es]
    for j in range(NB):
        cols = pl.ds(j * 128, 128)
        acc = es[0] * v_ref[pl.ds(kr, 16), cols]
        for w in range(1, WIN):
            acc = acc + es[w] * v_ref[pl.ds(kr - 8 * w, 16), cols]
        if 'P' not in EXP:
            acc = acc * inv
        word = pltpu.bitcast(acc.astype(BF16), U32)
        o_ref[pl.ds(qr // 2, 8), cols] = word
        done.append(pltpu.bitcast(acc, U32) if 'U' in EXP else word)
    return _token(done)


def _fill_halo(cur, prev, first, c0, width):
    cols = pl.ds(c0, width)
    sub = jax.lax.broadcasted_iota(I32, (8, width), 0)
    pos0 = jnp.broadcast_to(cur[pl.ds(WIN * 8, 1), cols], (8, width))
    for par in range(2):
        for g in range(1, WIN):
            src = pl.ds(par * KP + (NA + g) * 8, 8)
            if isinstance(first, bool):
                tail = pos0 if first else prev[src, cols]
            else:
                tail = jnp.where(first, pos0, prev[src, cols])
            cur[pl.ds(par * KP + g * 8, 8), cols] = pltpu.roll(jnp.where(sub == 7, tail, cur[src, cols]), 1, 0)


def _kernel(x_hbm, wa_hbm, woa_hbm, wb_hbm, wob_hbm, out_hbm,
            xin, xs, wraw, woraw, wq, wo, obuf,
            xn0, xn1, q0, q1, k0, k1, v0, v1, o0, o1, flag, isem, qsem, osem):
    xn, qb, kb, vb, ob = (xn0, xn1), (q0, q1), (k0, k1), (v0, v1), (o0, o1)

    def x_copy(t0, t1, sem):
        rows = pl.ds(t0 * TM, (t1 - t0) * TM)
        return pltpu.make_async_copy(x_hbm.at[rows], xin.at[rows], isem.at[sem])

    def wa_copy(sec):
        cols = pl.ds(sec * D, D)
        return pltpu.make_async_copy(wa_hbm.at[:, cols], wraw.at[0, :, cols], isem.at[sec])

    def wq_copy(c):
        rows = pl.ds(aligned(c * QR, QR), QR)
        return pltpu.make_async_copy(wa_hbm.at[rows, pl.ds(0, D)], wraw.at[0, rows, pl.ds(0, D)], qsem.at[c])

    x0_copy, x1_copy, xrest_copy = x_copy(0, 1, 3), x_copy(1, 2, 4), x_copy(2, NT, 5)
    woa_copy = pltpu.make_async_copy(woa_hbm, woraw.at[0], isem.at[6])
    wb_copy = pltpu.make_async_copy(wb_hbm, wraw.at[1], isem.at[7])
    wob_copy = pltpu.make_async_copy(wob_hbm, woraw.at[1], isem.at[8])

    def out_copy(t):
        return pltpu.make_async_copy(obuf.at[pl.ds(t * TM, TM)], out_hbm.at[pl.ds(t * TM, TM)], osem.at[t])

    def aligned(v, m):
        return v if isinstance(v, int) else pl.multiple_of(v, m)

    def tile(ref, t, c, width):
        return ref.at[pl.ds(_aligned(t * TM, TM), TM), pl.ds(_aligned(c * width, width), width)]

    def load_x(t, c, width):
        return _load_x(tile(xin, t, c, width), tile(xs, t, c, width))

    def load_x_tasks(t):
        return [functools.partial(load_x, t, c, 256) for c in range(D // 256)]

    def prep_wqkv_tasks(sec, rows=PREP_ROWS):
        return [functools.partial(_prep_wqkv, wraw.at[0], wq.at[0], r, rows, sec) for r in range(0, D // 2, rows)]

    def prep_wo_tasks():
        return [functools.partial(_prep_wo, woraw.at[0], wo.at[0], part) for part in range(4 * NB)]

    def ln_rows(row0, par, r, rows):
        y = _ln_rows(xs[pl.ds(row0 + r, rows), :])
        words = pltpu.bitcast(y.astype(BF16), U32)
        xn[par][pl.ds(aligned(r // 2, rows // 2), rows // 2), :] = words
        return _token([pltpu.bitcast(y, U32) if 'V' in EXP else words])

    def ln_tasks(i, par, rows=32):
        row0 = aligned((i % NT) * TM, TM)
        return [lambda r=r: ln_rows(row0, par, r, rows) for r in range(0, TM, rows)]

    def matmul(lhs, w, tokens):
        for half, ts in enumerate(tokens):
            if ts:
                r = half * (D // 4)
                corner = w[r:r + 8, :128]
                for t in ts:
                    corner = jnp.where(zero[0], t, corner)
                rows = [w[:r], jnp.concatenate([corner, w[r:r + 8, 128:]], axis=1), w[r + 8:]]
                w = jnp.concatenate(rows if half else rows[1:], axis=0)
        w = pltpu.bitcast(w, BF16)
        if 'M' in EXP and lhs.shape[0] == TM // 2:
            return jnp.concatenate([jnp.dot(pltpu.bitcast(lhs[m:m + TM // 4], BF16), w, preferred_element_type=F32)
                                    for m in (0, TM // 4)], axis=0)
        return jnp.dot(pltpu.bitcast(lhs, BF16), w, preferred_element_type=F32)

    def qkv_tasks(i, par):
        wsel = (i // NT) % 2
        first = (i % NT) == 0

        def f(c, tokens):
            r = matmul(xn[par][...], wq[wsel, :, c * NC:(c + 1) * NC], tokens)
            sec, c0 = divmod(c * NC, D)
            if sec == 0:
                qb[par][:, c0:c0 + NC] = r
            else:
                buf = kb if sec == 1 else vb
                for p in range(2):
                    buf[par][pl.ds(p * KP + WIN * 8, NA * 8), c0:c0 + NC] = r[p * NA * 8:(p + 1) * NA * 8]
                prev = buf[par] if first is True else buf[1 - par]
                _fill_halo(buf[par], prev, first if par == 0 else False, c0, NC)
        return [functools.partial(f, c) for c in range(3 * D // NC)]

    def proj_tasks(i, par):
        wsel = (i // NT) % 2
        row0 = aligned((i % NT) * TM, TM)

        def f(c, tokens):
            cols = slice(c * NC, (c + 1) * NC)
            r = matmul(ob[par][...], wo[wsel, :, cols], tokens)
            xs[pl.ds(row0, TM), cols] = xs[pl.ds(row0, TM), cols] + r
        return [functools.partial(f, c) for c in range(D // NC)]

    def final_proj_tasks(t, par, ah):
        def f(c, tokens):
            cols = slice(c * NC, (c + 1) * NC)
            lhs = jnp.concatenate([ob[par][pl.ds((p * NA + ah * 8) * 4, 32), :] for p in range(2)], axis=0)
            r = matmul(lhs, wo[1, :, cols], tokens)
            even, odd = [xs[pl.ds(t * TM + (p * NA + ah * 8) * 8, 64), cols] + r[p * 64:(p + 1) * 64]
                         for p in range(2)]
            return _store_out(even, odd, tile(obuf, t, c, NC), ah)
        return [functools.partial(f, c) for c in range(D // NC)]

    def attn_tasks(i, par):
        first = (i % NT) == 0 if par == 0 else False
        return [functools.partial(_attn_rows, qb[par], kb[par], vb[par], ob[par], p, a0, first)
                for p in range(2) for a0 in range(0, NA, 2)]

    LAG = 1
    ALAG = float(os.environ.get('LAG', 1))

    def spread(lo, hi, ts):
        return [(lo + k * (hi - lo) // len(ts), lo + k * (hi - lo) // len(ts) + LAG, f) for k, f in enumerate(ts)]

    def run(mms, *lists):
        n = len(mms)
        due = [[] for _ in range(2 * n + 1)]
        for c in range(n):
            token = mms[c](due[2 * c:2 * c + 2])
            if token is not None:
                due[min(2 * c + 4, 2 * n)].append(token)
            for at, before, f in [t for ts in lists for t in ts]:
                if at == c:
                    due[min(int(2 * before), 2 * n)].append(f())

    def loop(n, body):
        pl.loop(0, n)(lambda r: (body(r), None)[1])

    def ln_loop(t, par):
        loop(2, lambda c: [ln_rows(t * TM, par, pl.multiple_of(c * (TM // 2) + r, 32), 32)
                           for r in range(0, TM // 2, 32)])

    per = D // NC
    flag[0] = 0
    zero = [None]
    qkv0, qkv1 = qkv_tasks(0, 0), qkv_tasks(1, 1)
    def fill():
        x0_copy.start()
        wq_copy(0).start()
        x0_copy.wait()
        wq_copy(1).start()
        loop(D // 256, lambda c: load_x(0, c, 256))
        ln_loop(0, 0)

        mats = {j: _lane_matrix(j) for j in MQ}

        def prep_q(c):
            wq_copy(c).wait()

            @pl.when(c + 2 < NQ)
            def _():
                wq_copy(c + 2).start()

            @pl.when(c + 2 == NQ)
            def _():
                x1_copy.start()
                wa_copy(1).start()

            _prep_wqkv(wraw.at[0], wq.at[0], c * (QR // 2), QR // 2, 0, mats)
        loop(NQ, prep_q)
        wa_copy(2).start()
        x1_copy.wait()
        zero[0] = flag[0] != 0
        run(qkv0[:per], spread(0, per - 1, load_x_tasks(1) + ln_tasks(1, 1)))
        wa_copy(1).wait()
        woa_copy.start()
        run(qkv1[:per] + qkv0[per:2 * per], spread(0, per - 1, prep_wqkv_tasks(1)))
        wa_copy(2).wait()
        woa_copy.wait()
        xrest_copy.start()
        run(qkv1[per:2 * per] + qkv0[2 * per:] + qkv1[2 * per:], spread(0, per - 1, prep_wqkv_tasks(2)),
            spread(per - 1, 2 * per, prep_wo_tasks()), spread(2 * per, 3 * per - 1, attn_tasks(0, 0)))
        xrest_copy.wait()
        loop((NT - 2) * 2, lambda r: load_x(2 + (r >> 1), r & 1, 512))
        ln_loop(2, 0)

    if 'Z' not in EXP: fill()
    n = NL * NT

    def body(ii):
        @pl.when(ii == 0)
        def _():
            wb_copy.start()
            wob_copy.start()

        @pl.when(ii == 2)
        def _():
            wb_copy.wait()
            wob_copy.wait()

            mats = {j: _lane_matrix(j) for j in MX}

            def prep(r):
                _prep_wqkv(wraw.at[1], wq.at[1], (r & 3) * 128, 128, r >> 2, mats)
                for k in range(3):
                    _prep_wo(woraw.at[1], wo.at[1], jnp.minimum(3 * r + k, 4 * NB - 1))
            loop(12, prep)

        zero[0] = flag[0] != 0
        mms, att, lns = [], [], []
        for par in range(2):
            i = 2 + 2 * ii + par
            mms += qkv_tasks(i, par) + proj_tasks(i - 2, par)
            att += attn_tasks(i - 1, 1 - par)
            LD = [float(v) for v in os.environ.get('LD', '1,2,3,4,5,7,9,11').split(',')]
            ln = ln_tasks(i + 1, 1 - par, TM // len(LD))
            lns += [(par * 16 + min(int(d - float(os.environ.get('LL', 1))), 11), par * 16 + d, f) for d, f in zip(LD, ln)]
        run(mms, [(k, k + ALAG, f) for k, f in enumerate(att)], lns)

        @pl.when(ii >= (n - NT) // 2)
        def _():
            t0 = (2 * ii) % NT

            def conv(r):
                src, dst = [tile(ref, t0 + (r >> 2), r & 3, 256) for ref in (xs, obuf)]
                for ah in range(NA // 8):
                    _store_out(src[pl.ds(ah * 64, 64), :], src[pl.ds(NA * 8 + ah * 64, 64), :], dst, ah)
            loop(8, conv)
            out_copy(t0).start()
            out_copy(t0 + 1).start()

    loop(n // 2 - 1, body)
    if 'Z' in EXP:
        for t in range(NT - 2):
            out_copy(t).wait()
        return

    zero[0] = flag[0] != 0
    att = attn_tasks(n - 1, 1)
    att = att[:4] + att[8:12] + att[4:8] + att[12:]
    run(final_proj_tasks(NT - 2, 0, 0) + final_proj_tasks(NT - 2, 0, 1) + final_proj_tasks(NT - 1, 1, 0)
        + final_proj_tasks(NT - 1, 1, 1),
        spread(0, 8, att[:8]), spread(8, 12, att[8:]))
    out_copy(NT - 2).start()
    out_copy(NT - 1).start()
    for t in range(NT):
        out_copy(t).wait()


@jax.jit
def pallas_interleave_layers__sliding_local_dilated__sliding_local_dilated__prompt_kernel(
    A_x: jax.Array,
    A_wqkv: jax.Array,
    A_wo: jax.Array,
    B_x: jax.Array,
    B_wqkv: jax.Array,
    B_wo: jax.Array,
):
    del B_x
    any_spec = pl.BlockSpec(memory_space=pl.ANY)
    packed_tile = pltpu.VMEM((TM // 2, D), U32)
    q_tile = pltpu.VMEM((TM, D), F32)
    kv_tile = pltpu.VMEM((2 * KP, D), F32)
    out = pl.pallas_call(
        _kernel,
        in_specs=[any_spec] * 5,
        out_specs=any_spec,
        out_shape=jax.ShapeDtypeStruct((S, D), BF16),
        scratch_shapes=[
            pltpu.VMEM((S, D), BF16),
            pltpu.VMEM((S, D), F32),
            pltpu.VMEM((2, D, 3 * D), BF16),
            pltpu.VMEM((2, D, D), BF16),
            pltpu.VMEM((2, D // 2, 3 * D), U32),
            pltpu.VMEM((2, D // 2, D), U32),
            pltpu.VMEM((S, D), BF16),
            packed_tile, packed_tile, q_tile, q_tile,
            kv_tile, kv_tile, kv_tile, kv_tile, packed_tile, packed_tile,
            pltpu.SMEM((1,), I32),
            pltpu.SemaphoreType.DMA((9,)),
            pltpu.SemaphoreType.DMA((NQ,)),
            pltpu.SemaphoreType.DMA((NT,)),
        ],
        compiler_params=pltpu.CompilerParams(vmem_limit_bytes=100 * 1024 * 1024),
    )(A_x.reshape(S, D), A_wqkv, A_wo, B_wqkv, B_wo)
    return out.reshape(1, S, D)
```

```python
import functools

import jax
import jax.numpy as jnp
import jax.experimental.pallas as pl
import jax.experimental.pallas.tpu as pltpu
import numpy as np

S, D = 2048, 1024
H, DH = 32, 32
WIN = 8
NL = 4
NB = D // 128
TM = 256
NT = S // TM
NA = TM // 16
KP = (NA + WIN) * 8
NC = 256
PER = D // NC
NQ = 4
QR = D // NQ
MXU_BLOCKS = (1, 3, 5, 7)
LN_DUE = (1, 2, 3, 4, 5, 7, 9, 11)
LN_EPS = 1e-5
SCALE = DH ** -0.5
LOG2E = 1.4426950408889634
HI16, LO16 = np.uint32(0xFFFF0000), np.uint32(0xFFFF)
F32, BF16, U32, I32 = jnp.float32, jnp.bfloat16, jnp.uint32, jnp.int32


def _aligned(v, m):
    return v if isinstance(v, int) else pl.multiple_of(v, m)


def _token(words):
    return functools.reduce(jnp.bitwise_or, [
        w if w.shape == (8, 128) else w[a:a + 8, b:b + 128]
        for w in words for a in range(0, w.shape[0], 8) for b in range(0, w.shape[1], 128)])


def _xor_shuffle(t, masks):
    t = list(t)
    for b, m in masks.items():
        for ia in range(len(t)):
            if not ia & b:
                lo, hi = t[ia], t[ia | b]
                t[ia], t[ia | b] = jnp.where(m, hi, lo), jnp.where(m, lo, hi)
    return t


def _transpose8(slabs):
    sub = jax.lax.broadcasted_iota(I32, slabs[0].shape, 0)
    t = list(slabs)
    for b in (1, 2, 4):
        m = (sub & b) != 0
        for ia in range(8):
            if not ia & b:
                lo, hi = t[ia], t[ia | b]
                t[ia] = jnp.where(m, pltpu.roll(hi, b, 0), lo)
                t[ia | b] = jnp.where(m, hi, pltpu.roll(lo, 8 - b, 0))
    return t


def _lane_source(lane, j):
    dt, hh, hl = lane >> 5, (lane >> 2) & 7, lane & 3
    return hl * 32 + dt * 8 + (hh ^ j)


def _lane_matrices():
    src, lane = [jax.lax.broadcasted_iota(I32, (128, 128), axis) for axis in range(2)]
    return {j: jnp.where(src == _lane_source(lane, j), 1.0, 0.0).astype(BF16) for j in MXU_BLOCKS}


def _prep_wqkv(raw_ref, dst_ref, r0, rows, sec, mats=()):
    cols = pl.ds(_aligned(sec * D, D), D)
    raw = raw_ref.at[pl.ds(_aligned(2 * r0, 2 * rows), 2 * rows), cols]
    dst = dst_ref.at[pl.ds(_aligned(r0, rows), rows), cols]
    lane = jax.lax.broadcasted_iota(I32, (rows, 128), 1)
    t = _xor_shuffle([pltpu.bitcast(raw[:, j * 128:(j + 1) * 128], I32) for j in range(NB)],
                     {b: (lane & b) != 0 for b in (1, 2, 4)})
    blks = []
    for j in range(NB):
        if j in mats:
            blk = jnp.dot(pltpu.bitcast(t[j], BF16), mats[j], preferred_element_type=F32).astype(BF16)
        else:
            blk = jnp.take_along_axis(t[j], _lane_source(lane, j), axis=1)
        blks.append(pltpu.bitcast(blk, U32))
    for j, blk in enumerate(blks):
        dst[:, j * 128:(j + 1) * 128] = blk
    return _token(blks)


def _prep_wo(raw_ref, dst_ref, part):
    cols = pl.ds(_aligned((part >> 2) * 128, 128), 128)
    h4, d4 = (part >> 1) & 1, part & 1
    raw = raw_ref.at[pl.ds(_aligned(h4 * (D // 2) + d4 * 16, 16), D // 2 - 16), cols]
    dst = [dst_ref.at[pl.ds(_aligned((h4 ^ d2) * 256 + d4 * 32 + h4 * 8, 8), 216), cols] for d2 in range(2)]
    sub = jax.lax.broadcasted_iota(I32, (8, 128), 0)
    ev, od = [_transpose8([pltpu.bitcast(raw[pl.ds((hm * 2 + h0) * DH, 16), :], U32) for hm in range(8)])
              for h0 in range(2)]
    words = []
    for dm in range(8):
        words += [(ev[dm] & LO16) | (od[dm] << 16), (ev[dm] >> 16) | (od[dm] & HI16)]
    words = _xor_shuffle(words, {1: (sub & 2) != 0, 2: (sub & 4) != 0})
    for n, word in enumerate(words):
        dst[(n >> 2) & 1][pl.ds((n & 3) * 64 + (n >> 3) * 16, 8), :] = word
    return _token(words)


def _load_x(src, dst):
    done = []
    for ah in range(NA // 8):
        t = _transpose8([pltpu.bitcast(src[pl.ds((s * (NA // 8) + ah) * 16, 16), :], U32) for s in range(8)])
        for al in range(8):
            a = ah * 8 + al
            dst[pl.ds(a * 8, 8), :] = pltpu.bitcast(t[al] << 16, F32)
            dst[pl.ds((NA + a) * 8, 8), :] = pltpu.bitcast(t[al] & HI16, F32)
        done += t
    return _token(done)


def _store_out(even, odd, dst, ah):
    words = pltpu.pack_elementwise([even, odd], packed_dtype=BF16)
    t = _transpose8([words[al * 8:(al + 1) * 8] for al in range(8)])
    for s in range(8):
        dst[pl.ds((s * (NA // 8) + ah) * 16, 16), :] = pltpu.bitcast(t[s], BF16)
    return _token(t)


def _layernorm(x):
    c = x - jnp.mean(x, axis=-1, keepdims=True)
    v = jnp.mean(c * c, axis=-1, keepdims=True)
    return c * jax.lax.rsqrt(v + LN_EPS)


def _attention(q_ref, k_ref, v_ref, o_ref, par, a0, first):
    qr = (par * NA + a0) * 8
    kr = par * KP + (WIN + a0) * 8
    ls = [None] * WIN
    for j in range(NB):
        cols = pl.ds(j * 128, 128)
        q = q_ref[pl.ds(qr, 16), cols]
        for w in range(WIN):
            p = q * k_ref[pl.ds(kr - 8 * w, 16), cols]
            ls[w] = p if j == 0 else ls[w] + p
    row = jax.lax.broadcasted_iota(I32, (16, 128), 0)
    for w in range(WIN):
        l = ls[w]
        l = l + pltpu.roll(l, 64, 1)
        l = l + pltpu.roll(l, 32, 1)
        if w > a0 and first is not False:
            hit = (row == 0) if w == a0 + 1 else ((row & 7) == 0)
            l = jnp.where(hit if first is True else jnp.logical_and(hit, first), -1e9 / SCALE, l)
        ls[w] = l
    m = functools.reduce(lambda a, b: jnp.maximum(a, b), ls)
    es = [jnp.exp2((l - m) * (SCALE * LOG2E)) for l in ls]
    inv = 1.0 / functools.reduce(lambda a, b: a + b, es)
    done = []
    for j in range(NB):
        cols = pl.ds(j * 128, 128)
        acc = es[0] * v_ref[pl.ds(kr, 16), cols]
        for w in range(1, WIN):
            acc = acc + es[w] * v_ref[pl.ds(kr - 8 * w, 16), cols]
        acc = acc * inv
        o_ref[pl.ds(qr // 2, 8), cols] = pltpu.bitcast(acc.astype(BF16), U32)
        done.append(pltpu.bitcast(acc, U32))
    return _token(done)


def _fill_halo(cur, prev, first, c0):
    cols = pl.ds(c0, NC)
    sub = jax.lax.broadcasted_iota(I32, (8, NC), 0)
    pos0 = jnp.broadcast_to(cur[pl.ds(WIN * 8, 1), cols], (8, NC))
    for par in range(2):
        for g in range(1, WIN):
            src = pl.ds(par * KP + (NA + g) * 8, 8)
            if isinstance(first, bool):
                tail = pos0 if first else prev[src, cols]
            else:
                tail = jnp.where(first, pos0, prev[src, cols])
            cur[pl.ds(par * KP + g * 8, 8), cols] = pltpu.roll(jnp.where(sub == 7, tail, cur[src, cols]), 1, 0)


def _spread(lo, hi, tasks):
    slots = [lo + k * (hi - lo) // len(tasks) for k in range(len(tasks))]
    return [(at, at + 1, task) for at, task in zip(slots, tasks)]


def _run(matmuls, *task_lists):
    n = len(matmuls)
    due = [[] for _ in range(n + 1)]
    for c in range(n):
        token = matmuls[c](due[c])
        if token is not None:
            due[min(c + 2, n)].append(token)
        for at, before, task in [t for tasks in task_lists for t in tasks]:
            if at == c:
                due[min(before, n)].append(task())


def _loop(n, body):
    pl.loop(0, n)(lambda r: (body(r), None)[1])


def _kernel(x_hbm, wa_hbm, woa_hbm, wb_hbm, wob_hbm, out_hbm,
            xin, xs, wraw, woraw, wq, wo, obuf, xn0, xn1, q0, q1, k0, k1, v0, v1, o0, o1,
            flag, isem, qsem, osem):
    xn, qb, kb, vb, ob = (xn0, xn1), (q0, q1), (k0, k1), (v0, v1), (o0, o1)
    n = NL * NT

    def tile(ref, t, c, width):
        return ref.at[pl.ds(_aligned(t * TM, TM), TM), pl.ds(_aligned(c * width, width), width)]

    def x_copy(t0, t1, sem):
        rows = pl.ds(t0 * TM, (t1 - t0) * TM)
        return pltpu.make_async_copy(x_hbm.at[rows], xin.at[rows], isem.at[sem])

    def wq_copy(c):
        rows = pl.ds(_aligned(c * QR, QR), QR)
        return pltpu.make_async_copy(wa_hbm.at[rows, pl.ds(0, D)], wraw.at[0, rows, pl.ds(0, D)], qsem.at[c])

    def wa_copy(sec):
        cols = pl.ds(sec * D, D)
        return pltpu.make_async_copy(wa_hbm.at[:, cols], wraw.at[0, :, cols], isem.at[sec])

    def out_copy(t):
        return pltpu.make_async_copy(obuf.at[pl.ds(t * TM, TM)], out_hbm.at[pl.ds(t * TM, TM)], osem.at[t])

    def last_copy(c):
        return pltpu.make_async_copy(tile(obuf, NT - 1, c, NC), tile(out_hbm, NT - 1, c, NC), qsem.at[c])

    x0_copy, x1_copy, x2_copy, xrest_copy = x_copy(0, 1, 3), x_copy(1, 2, 4), x_copy(2, 3, 0), x_copy(3, NT, 5)
    woa_copy = pltpu.make_async_copy(woa_hbm, woraw.at[0], isem.at[6])
    wb_copy = pltpu.make_async_copy(wb_hbm, wraw.at[1], isem.at[7])
    wob_copy = pltpu.make_async_copy(wob_hbm, woraw.at[1], isem.at[8])

    flag[0] = 0
    never = [None]

    def matmul(lhs, w, tokens):
        if tokens:
            corner = w[:8, :128]
            for t in tokens:
                corner = jnp.where(never[0], t, corner)
            w = jnp.concatenate([jnp.concatenate([corner, w[:8, 128:]], axis=1), w[8:]], axis=0)
        return jnp.dot(pltpu.bitcast(lhs, BF16), pltpu.bitcast(w, BF16), preferred_element_type=F32)

    def load_x(t, c, width):
        return _load_x(tile(xin, t, c, width), tile(xs, t, c, width))

    def load_x_tasks(t):
        return [functools.partial(load_x, t, c, 256) for c in range(D // 256)]

    def prep_wqkv_tasks(sec):
        return [functools.partial(_prep_wqkv, wraw.at[0], wq.at[0], r, 64, sec) for r in range(0, D // 2, 64)]

    def prep_wo_tasks():
        return [lambda p0=p0: _token([_prep_wo(woraw.at[0], wo.at[0], p) for p in range(p0, p0 + 8)])
                for p0 in range(0, 4 * NB, 8)]

    def ln_rows(row0, par, r):
        words = pltpu.bitcast(_layernorm(xs[pl.ds(row0 + r, 32), :]).astype(BF16), U32)
        xn[par][pl.ds(_aligned(r // 2, 16), 16), :] = words
        return _token([words])

    def ln_tasks(i, par):
        row0 = _aligned((i % NT) * TM, TM)
        return [functools.partial(ln_rows, row0, par, r) for r in range(0, TM, 32)]

    def qkv_tasks(i, par):
        layer = (i // NT) % 2
        first = (i % NT) == 0 if par == 0 else False

        def f(c, tokens):
            r = matmul(xn[par][...], wq[layer, :, c * NC:(c + 1) * NC], tokens)
            sec, c0 = divmod(c * NC, D)
            if sec == 0:
                qb[par][:, c0:c0 + NC] = r
            else:
                buf = kb if sec == 1 else vb
                for p in range(2):
                    buf[par][pl.ds(p * KP + WIN * 8, NA * 8), c0:c0 + NC] = r[p * NA * 8:(p + 1) * NA * 8]
                _fill_halo(buf[par], buf[1 - par], first, c0)
        return [functools.partial(f, c) for c in range(3 * PER)]

    def proj_tasks(i, par):
        layer = (i // NT) % 2
        row0 = _aligned((i % NT) * TM, TM)

        def f(c, tokens):
            cols = slice(c * NC, (c + 1) * NC)
            r = matmul(ob[par][...], wo[layer, :, cols], tokens)
            xnew = xs[pl.ds(row0, TM), cols] + r
            xs[pl.ds(row0, TM), cols] = xnew
            for ah in range(NA // 8):
                _store_out(xnew[ah * 64:(ah + 1) * 64], xnew[NA * 8 + ah * 64:NA * 8 + (ah + 1) * 64],
                           tile(obuf, i % NT, c, NC), ah)
        return [functools.partial(f, c) for c in range(PER)]

    def final_proj_tasks(t, par, ah):
        def f(c, tokens):
            cols = slice(c * NC, (c + 1) * NC)
            lhs = jnp.concatenate([ob[par][pl.ds((p * NA + ah * 8) * 4, 32), :] for p in range(2)], axis=0)
            r = matmul(lhs, wo[(NL - 1) % 2, :, cols], tokens)
            even, odd = [xs[pl.ds(t * TM + (p * NA + ah * 8) * 8, 64), cols] + r[p * 64:(p + 1) * 64]
                         for p in range(2)]
            return _store_out(even, odd, tile(obuf, t, c, NC), ah)
        return [functools.partial(f, c) for c in range(PER)]

    def attn_tasks(i, par):
        first = (i % NT) == 0 if par == 0 else False
        return [functools.partial(_attention, qb[par], kb[par], vb[par], ob[par], p, a0, first)
                for p in range(2) for a0 in range(0, NA, 2)]

    qkv0, qkv1 = qkv_tasks(0, 0), qkv_tasks(1, 1)
    x0_copy.start()
    for c in range(NQ // 2):
        wq_copy(c).start()
    mats = _lane_matrices()
    x0_copy.wait()
    for c in range(NQ // 2, NQ):
        wq_copy(c).start()
    _loop(D // 256, lambda c: load_x(0, c, 256))
    _loop(2, lambda c: [ln_rows(0, 0, pl.multiple_of(c * (TM // 2) + r, 32)) for r in range(0, TM // 2, 32)])

    def prep_q(c):
        wq_copy(c).wait()

        @pl.when(c == 1)
        def _():
            x1_copy.start()
            wa_copy(1).start()

        _prep_wqkv(wraw.at[0], wq.at[0], c * (QR // 2), QR // 2, 0, mats)
    _loop(NQ, prep_q)
    wa_copy(2).start()
    x1_copy.wait()
    never[0] = flag[0] != 0
    _run(qkv0[:PER], _spread(0, PER - 1, load_x_tasks(1) + ln_tasks(1, 1)))
    wa_copy(1).wait()
    woa_copy.start()
    x2_copy.start()
    _run(qkv1[:PER] + qkv0[PER:2 * PER], _spread(0, PER, prep_wqkv_tasks(1)))
    wa_copy(2).wait()
    woa_copy.wait()
    x2_copy.wait()
    xrest_copy.start()
    _run(qkv1[PER:2 * PER] + qkv0[2 * PER:] + qkv1[2 * PER:],
         _spread(0, PER, prep_wqkv_tasks(2)),
         _spread(PER - 1, PER, [lambda: _token([task() for task in load_x_tasks(2)])]),
         _spread(PER, 2 * PER, prep_wo_tasks()),
         _spread(2 * PER, 3 * PER, ln_tasks(2, 0)),
         _spread(2 * PER, 3 * PER, attn_tasks(0, 0)))
    xrest_copy.wait()
    _loop((NT - 3) * 2, lambda r: load_x(3 + (r >> 1), r & 1, 512))

    def two_steps(ii):
        @pl.when(ii == 0)
        def _():
            wb_copy.start()
            wob_copy.start()

        @pl.when(ii == 2)
        def _():
            wb_copy.wait()
            wob_copy.wait()
            mats = _lane_matrices()

            def prep(rr):
                for r in (2 * rr, 2 * rr + 1):
                    for r0 in (0, 64):
                        _prep_wqkv(wraw.at[1], wq.at[1], (r & 3) * 128 + r0, 64, r >> 2, mats)
                    for k in range(3):
                        _prep_wo(woraw.at[1], wo.at[1], jnp.minimum(3 * r + k, 4 * NB - 1))
            _loop(6, prep)

        never[0] = flag[0] != 0
        matmuls, attn, ln = [], [], []
        for par in range(2):
            i = 2 + 2 * ii + par
            matmuls += qkv_tasks(i, par) + proj_tasks(i - 2, par)
            attn += attn_tasks(i - 1, 1 - par)
            ln += [(par * 4 * PER + due - 1, par * 4 * PER + due, task)
                   for due, task in zip(LN_DUE, ln_tasks(i + 1, 1 - par))]
        _run(matmuls, _spread(0, len(matmuls), attn), ln)

        @pl.when(ii >= (n - NT) // 2)
        def _():
            out_copy((2 * ii) % NT).start()
            out_copy((2 * ii) % NT + 1).start()

    _loop(n // 2 - 1, two_steps)

    never[0] = flag[0] != 0
    attn = attn_tasks(n - 1, 1)
    copies = [(2 * PER - 1, 4 * PER, out_copy(NT - 2).start)]
    copies += [(3 * PER + c, 4 * PER, last_copy(c).start) for c in range(PER)]
    _run(final_proj_tasks(NT - 2, 0, 0) + final_proj_tasks(NT - 2, 0, 1)
         + final_proj_tasks(NT - 1, 1, 0) + final_proj_tasks(NT - 1, 1, 1),
         _spread(0, 6, attn[:4] + attn[8:12]), _spread(6, 11, attn[4:8] + attn[12:]), copies)
    for t in range(NT - 1):
        out_copy(t).wait()
    for c in range(PER):
        last_copy(c).wait()


@jax.jit
def pallas_interleave_layers__sliding_local_dilated__sliding_local_dilated__prompt_kernel(
    A_x: jax.Array,
    A_wqkv: jax.Array,
    A_wo: jax.Array,
    B_x: jax.Array,
    B_wqkv: jax.Array,
    B_wo: jax.Array,
):
    del B_x
    any_spec = pl.BlockSpec(memory_space=pl.ANY)
    packed_tile = pltpu.VMEM((TM // 2, D), U32)
    q_tile = pltpu.VMEM((TM, D), F32)
    kv_tile = pltpu.VMEM((2 * KP, D), F32)
    out = pl.pallas_call(
        _kernel,
        in_specs=[any_spec] * 5,
        out_specs=any_spec,
        out_shape=jax.ShapeDtypeStruct((S, D), BF16),
        scratch_shapes=[
            pltpu.VMEM((S, D), BF16),
            pltpu.VMEM((S, D), F32),
            pltpu.VMEM((2, D, 3 * D), BF16),
            pltpu.VMEM((2, D, D), BF16),
            pltpu.VMEM((2, D // 2, 3 * D), U32),
            pltpu.VMEM((2, D // 2, D), U32),
            pltpu.VMEM((S, D), BF16),
            packed_tile, packed_tile,
            q_tile, q_tile,
            kv_tile, kv_tile, kv_tile, kv_tile,
            packed_tile, packed_tile,
            pltpu.SMEM((1,), I32),
            pltpu.SemaphoreType.DMA((9,)),
            pltpu.SemaphoreType.DMA((NQ,)),
            pltpu.SemaphoreType.DMA((NT,)),
        ],
        compiler_params=pltpu.CompilerParams(vmem_limit_bytes=100 * 1024 * 1024),
    )(A_x.reshape(S, D), A_wqkv, A_wo, B_wqkv, B_wo)
    return out.reshape(1, S, D)
```
